```python
import os as _os
_os.environ.setdefault("JAX_PLATFORMS", "cpu")
import jax
import jax.numpy as jnp

def _softmax(x, axis=-1):
    return jax.nn.softmax(x, axis=axis)
def _gelu(x):
    return jax.nn.gelu(x, approximate=True)
def _silu(x):
    return jax.nn.silu(x)
def _sigmoid(x):
    return jax.nn.sigmoid(x)
def _layernorm(x, axis=-1, eps=1e-5):
    m = jnp.mean(x, axis=axis, keepdims=True)
    v = jnp.var(x, axis=axis, keepdims=True)
    return (x - m) / jnp.sqrt(v + eps)
def _scatter_add(tgt, idx, src, axis=0):
    return tgt.at[idx].add(src)
def _segment_sum(src, seg, n):
    return jax.ops.segment_sum(src, seg, n)
class _Rng:
    def __init__(self, key):
        self._k = key
    def _next(self):
        self._k, sub = jax.random.split(self._k)
        return sub
    def normal(self, shape):
        return jax.random.normal(self._next(), shape, dtype=jnp.bfloat16)
    def randint(self, lo, hi, shape):
        return jax.random.randint(self._next(), shape, lo, hi, dtype=jnp.int32)
    def uniform(self, shape, lo=0.0, hi=1.0):
        return jax.random.uniform(self._next(), shape, jnp.bfloat16, lo, hi)
    def permutation(self, n):
        return jax.random.permutation(self._next(), n)


kernel_name = 'sequential_preLN__mha_block__dense_activation_mish__prompt'

def setup_inputs():
    _rng = _Rng(jax.random.key(int.from_bytes(__import__("os").urandom(4), "little")))
    _w = (lambda a: (lambda t: t.astype(jnp.bfloat16) if jnp.issubdtype(t.dtype, jnp.floating) else t)(jnp.asarray(a)))
    def _A_setup():
        B, S, D, H = 1, 2048, 576, 32
        return {
            "x": _w((lambda *s: _rng.normal(s) * 0.05)(B, S, D)),
            "wqkv": _w((lambda *s: _rng.normal(s) * 0.05)(D, 3 * D)),
            "wo": _w((lambda *s: _rng.normal(s) * 0.05)(D, D)),
        }
    _A_in = _A_setup()

    def _B_setup():
        B, S, D, F = 1, 2048, 576, 4608
        return {
            "x": _w((lambda *s: _rng.normal(s) * 0.05)(B, S, D)),
            "w1": _w((lambda *s: _rng.normal(s) * 1.6)(D, F) * (D ** -0.5)),
            "b1": _w((lambda *s: _rng.normal(s) * 0.05)(F)),
            "w2": _w((lambda *s: _rng.normal(s) * 0.05)(F, D) * (F ** -0.5)),
        }
    _B_in = _B_setup()

    return {
        "A_x": _A_in["x"],
        "A_wqkv": _A_in["wqkv"],
        "A_wo": _A_in["wo"],
        "B_x": _B_in["x"],
        "B_w1": _B_in["w1"],
        "B_b1": _B_in["b1"],
        "B_w2": _B_in["w2"],
    }

def reference(A_x, A_wqkv, A_wo, B_x, B_w1, B_b1, B_w2):
    def _A_ref(x, wqkv, wo):
        B, S, D = x.shape
        H = 32
        Dh = D // H
        qkv = (lambda x, *d: x.transpose(*d))((x @ wqkv).reshape(B, S, 3, H, Dh), 2, 0, 3, 1, 4)
        q, k, v = qkv[0], qkv[1], qkv[2]
        scores = jnp.einsum("bhqd,bhkd->bhqk", q, k) * (Dh ** -0.5)
        p = _softmax(scores, axis=-1)
        o = jnp.einsum("bhqk,bhkd->bhqd", p, v)
        return (lambda x, *d: x.transpose(*d))(o, 0, 2, 1, 3).reshape(B, S, D) @ wo

    def _B_ref(x, w1, b1, w2):
        h = jnp.einsum("bsd,df->bsf", x, w1) + b1
        sp = jnp.log1p(jnp.exp(-jnp.abs(h))) + jnp.where(h > 0, h, jnp.zeros_like(h))
        act = h * jnp.tanh(sp)
        return jnp.einsum("bsf,fd->bsd", act, w2)

    x = A_x
    h = x + _A_ref(_layernorm(x, axis=-1), A_wqkv, A_wo)
    h2 = h + _B_ref(_layernorm(h, axis=-1), B_w1, B_b1, B_w2)
    return h2
```

```python
import functools
import contextlib
import numpy as np
import jax
import jax.numpy as jnp
import jax.experimental.pallas as pl
import jax.experimental.pallas.tpu as pltpu

S, D, H, DH, F = 2048, 576, 32, 18, 4608
EPS = 1e-5
LOG2E = 1.4426950408889634
HS = 20
HPW = 7
NW = 5
f32, bf16 = jnp.float32, jnp.bfloat16


def _ln_t(xT):
    m = jnp.sum(xT, axis=0, keepdims=True) * (1.0 / D)
    xc = xT - m
    v = jnp.sum(xc * xc, axis=0, keepdims=True) * (1.0 / D)
    return xc * jax.lax.rsqrt(v + EPS)


def _mish(h):
    t = jnp.exp2(jnp.minimum(h, 20.0) * LOG2E)
    n = t * (t + 2.0)
    return h * (n / (n + 2.0))


def _nt(a, b):
    return jax.lax.dot_general(a, b, (((1,), (1,)), ((), ())), preferred_element_type=f32)


def _tn(a, b):
    return jax.lax.dot_general(a, b, (((0,), (0,)), ((), ())), preferred_element_type=f32)


def make(BQ=512, G=8, FC=512, BP=512, name="fused", scopes=False, ytr="f32", FU=9, pvf32=True):
    BK = 128
    NK = S // BK
    NGRP = H // G
    GR = HS * G
    NQB = S // BQ
    NPB = S // BP
    QSCALE = LOG2E / np.sqrt(DH)
    HP = HS * H

    vdt = f32 if pvf32 else bf16
    def scope(n):
        return jax.named_scope(n) if scopes else contextlib.nullcontext()

    def tr(xT):
        if ytr == "f32":
            return xT.T.astype(bf16)
        return xT.astype(bf16).T

    def kernel(xT_hbm, wqkv_hbm, wo_hbm, w1_hbm, b1_ref, w2T_hbm, out_ref,
               xT_s, wqkv_s, wo_s, w1_s, w2T_s, wqk_s, wvt_s, woT_s, tmp_s, b1_s,
               q_s, k_s, vt_s, ot_s, acc_s, sems):
        i = pl.program_id(0)

        def cp_x(b):
            return pltpu.make_async_copy(xT_hbm.at[:, pl.ds(b * BP, BP)], xT_s.at[:, pl.ds(b * BP, BP)], sems.at[b])
        cp_wqkv = pltpu.make_async_copy(wqkv_hbm, wqkv_s, sems.at[NPB])
        cp_wo = pltpu.make_async_copy(wo_hbm, wo_s, sems.at[NPB + 1])
        cp_w1 = pltpu.make_async_copy(w1_hbm, w1_s, sems.at[NPB + 2])
        cp_w2 = pltpu.make_async_copy(w2T_hbm, w2T_s, sems.at[NPB + 3])

        @pl.when(i == 0)
        def _prologue():
            with scope("sc_start"):
                cp_wqkv.start()
                for b in range(NPB):
                    cp_x(b).start()
                cp_wo.start()
                cp_w1.start()
                cp_w2.start()
                cp_wqkv.wait()
            with scope("sc_relayout"):
                for t in range(2):
                    for g in range(NW):
                        c0 = D * t + HPW * DH * g
                        wqk_s[:, (NW * t + g) * 128:(NW * t + g + 1) * 128] = wqkv_s[:, c0:c0 + 128]
                wvT = wqkv_s[:, 2 * D:3 * D].astype(f32).T
                tmp_s[...] = jnp.zeros(tmp_s.shape, f32)
                for h in range(H):
                    tmp_s[HS * h:HS * h + DH, :] = wvT[DH * h:DH * h + DH, :]
                wvt_s[...] = tmp_s[...].astype(bf16)
                for c in range(F // 128):
                    b1_s[:, c * 128:(c + 1) * 128] = jnp.broadcast_to(b1_ref[c:c + 1, :].astype(f32), (8, 128))

            def proj(b, carry):
                cp_x(b).wait()
                r0 = pl.multiple_of(b * BP, BP)
                xnT = _ln_t(xT_s[:, pl.ds(r0, BP)].astype(f32))
                xn = tr(xnT)
                xnT = xnT.astype(bf16)
                vT = jnp.dot(wvt_s[...], xnT, preferred_element_type=f32)
                row = jax.lax.broadcasted_iota(jnp.int32, (GR, BP), 0)
                ones = jnp.where(row % HS == DH, 1.0, 0.0).astype(f32)
                for j in range(NGRP):
                    vt_s[j, :, pl.ds(r0, BP)] = (vT[j * GR:(j + 1) * GR, :] + ones).astype(vdt)
                qk = jnp.dot(xn, wqk_s[...], preferred_element_type=f32)
                for g in range(NW):
                    q_s[g, pl.ds(r0, BP), :] = (qk[:, g * 128:(g + 1) * 128] * QSCALE).astype(bf16)
                    k_s[g, pl.ds(r0, BP), :] = qk[:, (NW + g) * 128:(NW + g + 1) * 128].astype(bf16)
                return carry
            with scope("sc_proj"):
                jax.lax.fori_loop(0, NPB, proj, 0)

            with scope("sc_relayout2"):
                cp_wo.wait()
                wof = wo_s[...].astype(f32)
                for h in range(H):
                    tmp_s[HS * h:HS * h + DH, :] = wof[DH * h:DH * h + DH, :]
                woT_s[...] = tmp_s[...].T.astype(bf16)

        q0 = pl.multiple_of(i * BQ, BQ)

        def group(j, carry):
            steps = [(hh, kb) for hh in range(G) for kb in range(NK)]
            N = len(steps)
            qm = {}

            def head_info(hh):
                h = j * G + hh
                g = h // HPW
                return g, (h - g * HPW) * DH

            def getq(hh):
                if hh not in qm:
                    g, r0 = head_info(hh)
                    qw = pltpu.bitcast(q_s[g, pl.ds(q0, BQ), :], jnp.int32)
                    lane = jax.lax.broadcasted_iota(jnp.int32, (8, 128), 1)
                    msk = jnp.where((lane >= r0) & (lane < r0 + DH), -1, 0).astype(jnp.int32)
                    msk = jnp.broadcast_to(msk[None], (BQ // 16, 8, 128)).reshape(BQ // 2, 128)
                    qm[hh] = (g, pltpu.bitcast(qw & msk, bf16))
                return qm[hh]

            def A(n):
                hh, kb = steps[n]
                g, q = getq(hh)
                kk = k_s[g, kb * BK:(kb + 1) * BK, :]
                sT = _nt(kk, q)
                return sT, jnp.max(sT, axis=0, keepdims=True)

            def B(n, smx, m_run):
                hh, kb = steps[n]
                sT, mx = smx
                if kb == 0:
                    m_new, alpha = mx, None
                else:
                    m_new = jnp.maximum(m_run, mx)
                    alpha = jnp.exp2(m_run - m_new)
                p = jnp.exp2(sT - m_new).astype(vdt)
                return p, alpha, m_new

            def C(n, p, alpha, acc):
                hh, kb = steps[n]
                st = (8 * ((HS * hh) // 8)) if pvf32 else (16 * ((HS * hh) // 16))
                off = HS * hh - st
                vT = vt_s[j, st:st + (24 if pvf32 else 32), kb * BK:(kb + 1) * BK]
                r = jnp.dot(vT, p, preferred_element_type=f32)
                acc = r if kb == 0 else acc * alpha + r
                if kb == NK - 1:
                    l = acc[off + DH:off + DH + 1, :]
                    ot_s[j, HS * hh:HS * hh + HS, :] = acc[off:off + HS, :] * pltpu.reciprocal(l, approx=False)
                return acc

            m_run = None
            acc = None
            As = {0: A(0), 1: A(1)}
            Bs = {}
            p, alpha, m_run = B(0, As.pop(0), m_run)
            Bs[0] = (p, alpha)
            for n in range(N):
                if n + 2 < N:
                    As[n + 2] = A(n + 2)
                if n + 1 < N:
                    p, alpha, m_run = B(n + 1, As.pop(n + 1), m_run)
                    Bs[n + 1] = (p, alpha)
                acc = C(n, *Bs.pop(n), acc)
            return carry

        with scope("sc_attn"):
            jax.lax.fori_loop(0, NGRP, group, 0)

        with scope("sc_wwait"):
            @pl.when(i == 0)
            def _():
                cp_w1.wait()
                cp_w2.wait()

        with scope("sc_dense"):
            oT = ot_s[...].reshape(HP, BQ).astype(bf16)
            attnT = jnp.dot(woT_s[...], oT, preferred_element_type=f32)
            hT = xT_s[:, pl.ds(q0, BQ)].astype(f32) + attnT
            y = tr(_ln_t(hT))

            def F1(c0):
                h1 = jnp.dot(y, w1_s[:, pl.ds(c0, FC)], preferred_element_type=f32)
                h1 = (h1.reshape(BQ // 8, 8, FC) + b1_s[:, pl.ds(c0, FC)][None]).reshape(BQ, FC)
                return _mish(h1).astype(bf16)

            NC = F // FC
            if FU == NC:
                acc = hT
                a = F1(0)
                for c in range(NC):
                    a_next = F1((c + 1) * FC) if c + 1 < NC else None
                    acc = acc + _nt(w2T_s[:, c * FC:(c + 1) * FC], a)
                    a = a_next
            else:
                acc_s[...] = hT
                def fbody(it, carry):
                    base = it * (FU * FC)
                    a = F1(pl.multiple_of(base, FC))
                    acc = acc_s[...]
                    for u in range(FU):
                        a_next = F1(pl.multiple_of(base + (u + 1) * FC, FC)) if u + 1 < FU else None
                        acc = acc + _nt(w2T_s[:, pl.ds(pl.multiple_of(base + u * FC, FC), FC)], a)
                        a = a_next
                    acc_s[...] = acc
                    return carry
                jax.lax.fori_loop(0, NC // FU, fbody, 0)
                acc = acc_s[...]
            out_ref[...] = acc.astype(bf16)

    hbm = pl.BlockSpec(memory_space=pltpu.HBM)
    call = pl.pallas_call(
        kernel,
        grid=(NQB,),
        in_specs=[hbm, hbm, hbm, hbm, pl.BlockSpec((F // 128, 128), lambda i: (0, 0)), hbm],
        out_specs=pl.BlockSpec((D, BQ), lambda i: (0, i)),
        out_shape=jax.ShapeDtypeStruct((D, S), bf16),
        scratch_shapes=[
            pltpu.VMEM((D, S), bf16),
            pltpu.VMEM((D, 3 * D), bf16),
            pltpu.VMEM((D, D), bf16),
            pltpu.VMEM((D, F), bf16),
            pltpu.VMEM((D, F), bf16),
            pltpu.VMEM((D, 2 * NW * 128), bf16),
            pltpu.VMEM((HP, D), bf16),
            pltpu.VMEM((D, HP), bf16),
            pltpu.VMEM((HP, D), f32),
            pltpu.VMEM((8, F), f32),
            pltpu.VMEM((NW, S, 128), bf16),
            pltpu.VMEM((NW, S, 128), bf16),
            pltpu.VMEM((NGRP, GR, S), vdt),
            pltpu.VMEM((NGRP, GR, BQ), f32),
            pltpu.VMEM((D, BQ), f32),
            pltpu.SemaphoreType.DMA((NPB + 4,)),
        ],
        compiler_params=pltpu.CompilerParams(
            dimension_semantics=("arbitrary",),
            vmem_limit_bytes=100 * 1024 * 1024,
        ),
        name=name,
    )

    @jax.jit
    def fn(A_x, A_wqkv, A_wo, B_x, B_w1, B_b1, B_w2):
        outT = call(A_x.reshape(S, D).T, A_wqkv, A_wo, B_w1, B_b1.reshape(F // 128, 128), B_w2.T)
        return outT.T.reshape(1, S, D)
    return fn


_impl = make(G=8, FU=3)


@jax.jit
def pallas_sequential_preLN__mha_block__dense_activation_mish__prompt_kernel(
    A_x: jax.Array,
    A_wqkv: jax.Array,
    A_wo: jax.Array,
    B_x: jax.Array,
    B_w1: jax.Array,
    B_b1: jax.Array,
    B_w2: jax.Array,
):
    return _impl(A_x, A_wqkv, A_wo, B_x, B_w1, B_b1, B_w2)
```

```python
import contextlib
import numpy as np
import jax
import jax.numpy as jnp
import jax.experimental.pallas as pl
import jax.experimental.pallas.tpu as pltpu

S, D, H, DH, F = 2048, 576, 32, 18, 4608
EPS = 1e-5
LOG2E = 1.4426950408889634
HS = 20
HPW = 7
NW = 5
f32, bf16 = jnp.float32, jnp.bfloat16


def _ln_t(xT):
    m = jnp.sum(xT, axis=0, keepdims=True) * (1.0 / D)
    xc = xT - m
    v = jnp.sum(xc * xc, axis=0, keepdims=True) * (1.0 / D)
    return xc * jax.lax.rsqrt(v + EPS)


def _mish(h):
    t = jnp.exp2(jnp.minimum(h, 20.0) * LOG2E)
    n = t * (t + 2.0)
    return h * (n / (n + 2.0))


def _nn(a, b):
    return jnp.dot(a, b, preferred_element_type=f32)


def _nt(a, b):
    return jax.lax.dot_general(a, b, (((1,), (1,)), ((), ())), preferred_element_type=f32)


def make(BQ=512, G=8, FC=512, FU=3, name="fused", scopes=False, outw=True, split=False, peel=3, carry=1, preq=True, p1=1, p2=1, p3=1):
    BK = 128
    NK = S // BK
    NGRP = H // G
    GR = HS * G
    NQB = S // BQ
    QSCALE = LOG2E / np.sqrt(DH)
    HP = HS * H
    NC = F // FC

    def scope(n):
        return jax.named_scope(n) if scopes else contextlib.nullcontext()

    def kernel(xT_hbm, wqkv_hbm, wo_hbm, w1_hbm, b1_hbm, w2T_hbm, out_ref,
               xT_s, wqkv_s, wo_s, w1_s, w2T_s, wqk_s, wvT_s, woT_s, tmp_s, b1_s,
               pad1, q_s, k_s, pad2, vt_s, ot_s, acc_s, sc_s, pc_s, mc_s, xn_s, xnT_s, b1r_s, pad3, sems):
        i = pl.program_id(0)

        def cp_x(b):
            return pltpu.make_async_copy(xT_hbm.at[:, pl.ds(b * BQ, BQ)], xT_s.at[:, pl.ds(b * BQ, BQ)], sems.at[b])
        C0 = 2 * D
        cp_wqk = pltpu.make_async_copy(wqkv_hbm.at[:, pl.ds(0, C0)], wqkv_s.at[:, pl.ds(0, C0)], sems.at[NQB])
        cp_wv = pltpu.make_async_copy(wqkv_hbm.at[:, pl.ds(C0, 3 * D - C0)], wqkv_s.at[:, pl.ds(C0, 3 * D - C0)], sems.at[NQB + 1])
        cp_wo = pltpu.make_async_copy(wo_hbm, wo_s, sems.at[NQB + 2])
        cp_w1 = pltpu.make_async_copy(w1_hbm, w1_s, sems.at[NQB + 3])
        cp_w2 = pltpu.make_async_copy(w2T_hbm, w2T_s, sems.at[NQB + 4])
        cp_b1 = pltpu.make_async_copy(b1_hbm, b1r_s, sems.at[NQB + 5])

        @pl.when(i == 0)
        def _prologue():
            with scope("sc_start"):
                cp_x(0).start()
                cp_wv.start()
                for b in range(1, NQB):
                    cp_x(b).start()
                cp_wqk.start()
                cp_wo.start()
                cp_b1.start()
                cp_w1.start()
                cp_w2.start()
                two = jnp.where(jax.lax.broadcasted_iota(jnp.int32, (2, S), 0) == 0, 1.0, 0.0)
                for h in range(H):
                    j, hh = divmod(h, G)
                    vt_s[j, HS * hh + DH:HS * hh + HS, :] = two
                    tmp_s[HS * h + DH:HS * h + HS, :] = jnp.zeros((HS - DH, D), f32)
                pad3[0:8, :] = jnp.zeros((8, 128), f32)
                pad1[0:8, :] = jnp.zeros((8, 128), f32)
                pad2[0:8, :] = jnp.zeros((8, 128), f32)
                cp_x(0).wait()

            def ln1(b):
                r0 = pl.multiple_of(b * BQ, BQ)
                xnT = _ln_t(xT_s[:, pl.ds(r0, BQ)].astype(f32))
                xn_s[b] = xnT.T.astype(bf16)
                xnT_s[b] = xnT.astype(bf16)

            def windows():
                tiles = {}

                def tile(a):
                    if a not in tiles:
                        tiles[a] = pltpu.bitcast(wqkv_s[:, a * 128:(a + 1) * 128], jnp.int32)
                    return tiles[a]
                lane = jax.lax.broadcasted_iota(jnp.int32, (D // 2, 128), 1)
                for t in range(2):
                    for g in range(NW):
                        c0 = D * t + HPW * DH * g
                        a, off = divmod(c0, 128)
                        if off == 0:
                            w = tile(a)
                        else:
                            w = pltpu.roll(jnp.where(lane >= off, tile(a), tile(a + 1)), 128 - off, 1)
                        wqk_s[:, (NW * t + g) * 128:(NW * t + g + 1) * 128] = pltpu.bitcast(w, bf16)

            def vproj(b):
                r0 = pl.multiple_of(b * BQ, BQ)
                vT = _nn(wvT_s[...], xnT_s[b])
                for h in range(H):
                    j, hh = divmod(h, G)
                    vt_s[j, HS * hh:HS * hh + DH, pl.ds(r0, BQ)] = vT[DH * h:DH * h + DH, :]

            def qkproj(b):
                r0 = pl.multiple_of(b * BQ, BQ)
                qk = _nn(xn_s[b], wqk_s[...])
                if preq:
                    r2 = pl.multiple_of(b * (BQ // 2), BQ // 2)
                    lane = jax.lax.broadcasted_iota(jnp.int32, (BQ // 2, 128), 1)
                    for g in range(NW):
                        qg = pltpu.bitcast((qk[:, g * 128:(g + 1) * 128] * QSCALE).astype(bf16), jnp.int32)
                        for h in range(g * HPW, min(H, (g + 1) * HPW)):
                            r = (h - g * HPW) * DH
                            q_s[h, pl.ds(r2, BQ // 2), :] = jnp.where((lane >= r) & (lane < r + DH), qg, 0)
                        k_s[g, pl.ds(r2, BQ // 2), :] = pltpu.bitcast(qk[:, (NW + g) * 128:(NW + g + 1) * 128].astype(bf16), jnp.int32)
                    return
                for g in range(NW):
                    q_s[g, pl.ds(r0, BQ), :] = (qk[:, g * 128:(g + 1) * 128] * QSCALE).astype(bf16)
                    k_s[g, pl.ds(r0, BQ), :] = qk[:, (NW + g) * 128:(NW + g + 1) * 128].astype(bf16)

            def wo_prep():
                wof = wo_s[...].astype(f32)
                for h in range(H):
                    tmp_s[HS * h:HS * h + DH, :] = wof[DH * h:DH * h + DH, :]
                woT_s[...] = tmp_s[...].T.astype(bf16)
                for c in range(F // 128):
                    b1_s[:, c * 128:(c + 1) * 128] = jnp.broadcast_to(b1r_s[c:c + 1, :].astype(f32), (8, 128))

            with scope("sc_ln0"):
                ln1(0)
                cp_wv.wait()
            with scope("sc_relayout"):
                wvT_s[...] = wqkv_s[:, 2 * D:3 * D].astype(f32).T.astype(bf16)

            def vloop(b, c):
                cp_x(b + 1).wait()
                vproj(b)
                ln1(b + 1)
                return c

            def qkloop(b, c):
                qkproj(b)
                return c

            with scope("sc_vproj"):
                jax.lax.fori_loop(0, NQB - 1, vloop, 0)
                cp_wqk.wait()
                if peel & 1:
                    vproj(NQB - 1)
                    windows()
                else:
                    windows()
                    jax.lax.fori_loop(NQB - 1, NQB, lambda b, c: (vproj(b), c)[1], 0) if False else vproj(NQB - 1)
            with scope("sc_qkproj"):
                if peel & 2:
                    jax.lax.fori_loop(0, NQB - 1, qkloop, 0)
                    cp_wo.wait()
                    cp_b1.wait()
                    qkproj(NQB - 1)
                    wo_prep()
                else:
                    jax.lax.fori_loop(0, NQB, qkloop, 0)
                    cp_wo.wait()
                    cp_b1.wait()
                    wo_prep()

        q0 = pl.multiple_of(i * BQ, BQ)

        def masked_q(j, qq0, hh):
            h = j * G + hh
            g = (h * 37) >> 8
            if preq:
                return (g, (h, pl.multiple_of(qq0 // 2, BQ // 2)))
            r0 = (h - g * HPW) * DH
            qw = pltpu.bitcast(q_s[g, pl.ds(qq0, BQ), :], jnp.int32)
            lane = jax.lax.broadcasted_iota(jnp.int32, (8, 128), 1)
            msk = jnp.where((lane >= r0) & (lane < r0 + DH), -1, 0).astype(jnp.int32)
            msk = jnp.broadcast_to(msk[None], (BQ // 16, 8, 128)).reshape(BQ // 2, 128)
            return (g, pltpu.bitcast(qw & msk, bf16))

        def A(gq, kb):
            g, q = gq
            if preq:
                h, r2 = q
                q = pltpu.bitcast(q_s[h, pl.ds(r2, BQ // 2), :], bf16)
                kk = pltpu.bitcast(k_s[g, kb * (BK // 2):(kb + 1) * (BK // 2), :], bf16)
                sT = _nt(kk, q)
            else:
                sT = _nt(k_s[g, kb * BK:(kb + 1) * BK, :], q)
            return sT, jnp.max(sT, axis=0, keepdims=True)

        def B(kb, smx, m_run):
            sT, mx = smx
            if kb == 0:
                m_new, alpha = mx, None
            else:
                m_new = jnp.maximum(m_run, mx)
                alpha = jnp.exp2(m_run - m_new)
            return jnp.exp2(sT - m_new), alpha, m_new

        def C(j, hh, kb, p, alpha, acc):
            st = 8 * ((HS * hh) // 8)
            off = HS * hh - st
            vT = vt_s[j, st:st + 24, kb * BK:(kb + 1) * BK]
            r = _nn(vT, p)
            acc = r if kb == 0 else acc * alpha + r
            if kb == NK - 1:
                l = acc[off + DH:off + DH + 1, :]
                ot_s[j, HS * hh:HS * hh + HS, :] = acc[off:off + HS, :] * pltpu.reciprocal(l, approx=False)
            return acc

        N = G * NK

        def group(j, c):
            last = j == NGRP - 1
            jn = jnp.where(last, 0, j + 1)
            q0n = pl.multiple_of(jnp.minimum(i + last.astype(jnp.int32), NQB - 1) * BQ, BQ)
            qm = {}

            def getq(n):
                key = n // NK
                if key not in qm:
                    qm[key] = masked_q(j, q0, key) if key < G else masked_q(jn, q0n, 0)
                return qm[key]
            if carry == 1:
                As = {1: (sc_s[...], mc_s[1:2, :])}
                Bs = {0: (pc_s[...], None)}
                m_run = mc_s[0:1, :]
            else:
                a0 = (sc_s[...], mc_s[1:2, :]) if carry == 3 else A(getq(0), 0)
                As = {1: A(getq(1), 1)}
                p, alpha, m_run = B(0, a0, None)
                Bs = {0: (p, alpha)}
            LIM = {0: N, 1: N + 2, 3: N + 1}[carry]
            acc = None
            for n in range(N):
                if n + 2 < LIM:
                    As[n + 2] = A(getq(n + 2), (n + 2) % NK)
                if n + 1 < N or carry == 1:
                    p, alpha, m_run = B((n + 1) % NK, As.pop(n + 1), m_run)
                    Bs[n + 1] = (p, alpha)
                acc = C(j, n // NK, n % NK, *Bs.pop(n), acc)
            if carry == 1:
                sT, mx = As.pop(N + 1)
                p, _ = Bs.pop(N)
                sc_s[...] = sT
                pc_s[...] = p
                mc_s[0:1, :] = m_run
                mc_s[1:2, :] = mx
            elif carry == 3:
                sT, mx = As.pop(N)
                sc_s[...] = sT
                mc_s[1:2, :] = mx
            return c

        with scope("sc_attn"):
            @pl.when(i == 0)
            def _():
                gq = masked_q(0, 0, 0)
                a0 = A(gq, 0)
                if carry == 3:
                    sc_s[...] = a0[0]
                    mc_s[1:2, :] = a0[1]
                else:
                    sT, mx = A(gq, 1)
                    p, _, m0 = B(0, a0, None)
                    sc_s[...] = sT
                    pc_s[...] = p
                    mc_s[0:1, :] = m0
                    mc_s[1:2, :] = mx
            jax.lax.fori_loop(0, NGRP, group, 0)

        with scope("sc_wwait"):
            @pl.when(i == 0)
            def _():
                cp_w1.wait()
                cp_w2.wait()

        with scope("sc_dense"):
            if not split:
                oT = ot_s[...].reshape(HP, BQ).astype(bf16)
                attnT = _nn(woT_s[...], oT)
            if split:
                HB = BQ // 2
                KM = 512
                xk = xT_s[:, pl.ds(q0, BQ)].astype(f32)
                oT = ot_s[...].reshape(HP, BQ).astype(bf16)
                d0 = _nn(woT_s[:, :KM], oT[:KM, :HB])
                dt = _nn(woT_s[:, KM:], oT[KM:, :])
                h0 = xk[:, :HB] + (d0 + dt[:, :HB])
                y0 = _ln_t(h0).T.astype(bf16)
                d1 = _nn(woT_s[:, :KM], oT[:KM, HB:])
                h1 = xk[:, HB:] + (d1 + dt[:, HB:])
                y1 = _ln_t(h1).T.astype(bf16)
                y = jnp.concatenate([y0, y1], axis=0)
                hT = jnp.concatenate([h0, h1], axis=1)
            else:
                hT = xT_s[:, pl.ds(q0, BQ)].astype(f32) + attnT
                y = _ln_t(hT).T.astype(bf16)

            def F1(c0):
                h1 = _nn(y, w1_s[:, pl.ds(c0, FC)])
                h1 = (h1.reshape(BQ // 8, 8, FC) + b1_s[:, pl.ds(c0, FC)][None]).reshape(BQ, FC)
                return _mish(h1).astype(bf16)

            acc_s[...] = hT

            def fbody(it, c):
                base = it * (FU * FC)
                a = F1(pl.multiple_of(base, FC))
                acc = acc_s[...]
                for u in range(FU):
                    a_next = F1(pl.multiple_of(base + (u + 1) * FC, FC)) if u + 1 < FU else None
                    acc = acc + _nt(w2T_s[:, pl.ds(pl.multiple_of(base + u * FC, FC), FC)], a)
                    a = a_next
                acc_s[...] = acc
                if outw:
                    out_ref[...] = acc.astype(bf16)
                return c
            jax.lax.fori_loop(0, NC // FU, fbody, 0)
            if not outw:
                out_ref[...] = acc_s[...].astype(bf16)

    hbm = pl.BlockSpec(memory_space=pltpu.HBM)
    V = pltpu.VMEM
    call = pl.pallas_call(
        kernel,
        grid=(NQB,),
        in_specs=[hbm] * 6,
        out_specs=pl.BlockSpec((D, BQ), lambda i: (0, i)),
        out_shape=jax.ShapeDtypeStruct((D, S), bf16),
        scratch_shapes=[
            V((D, S), bf16),
            V((D, 3 * D), bf16),
            V((D, D), bf16),
            V((D, F), bf16),
            V((D, F), bf16),
            V((D, 2 * NW * 128), bf16),
            V((D, D), bf16),
            V((D, HP), bf16),
            V((HP, D), f32),
            V((8, F), f32),
            V((8 * p1, 128), f32),
            V((H, S // 2, 128), jnp.int32) if preq else V((NW, S, 128), bf16),
            V((NW, S // 2, 128), jnp.int32) if preq else V((NW, S, 128), bf16),
            V((8 * p2, 128), f32),
            V((NGRP, GR, S), f32),
            V((NGRP, GR, BQ), f32),
            V((D, BQ), f32),
            V((BK, BQ), f32),
            V((BK, BQ), f32),
            V((8, BQ), f32),
            V((NQB, BQ, D), bf16),
            V((NQB, D, BQ), bf16),
            V((F // 128, 128), bf16),
            V((8 * p3, 128), f32),
            pltpu.SemaphoreType.DMA((NQB + 6,)),
        ],
        compiler_params=pltpu.CompilerParams(
            dimension_semantics=("arbitrary",),
            vmem_limit_bytes=100 * 1024 * 1024,
        ),
        name=name,
    )

    @jax.jit
    def fn(A_x, A_wqkv, A_wo, B_x, B_w1, B_b1, B_w2):
        outT = call(A_x.reshape(S, D).T, A_wqkv, A_wo, B_w1, B_b1.reshape(F // 128, 128), B_w2.T)
        return outT.T.reshape(1, S, D)
    return fn


_impl = make(carry=3)


@jax.jit
def pallas_sequential_preLN__mha_block__dense_activation_mish__prompt_kernel(
    A_x: jax.Array,
    A_wqkv: jax.Array,
    A_wo: jax.Array,
    B_x: jax.Array,
    B_w1: jax.Array,
    B_b1: jax.Array,
    B_w2: jax.Array,
):
    return _impl(A_x, A_wqkv, A_wo, B_x, B_w1, B_b1, B_w2)
```

```python
import numpy as np
import jax
import jax.numpy as jnp
import jax.experimental.pallas as pl
import jax.experimental.pallas.tpu as pltpu

S, D, H, DH, F = 2048, 576, 32, 18, 4608
EPS = 1e-5
LOG2E = 1.4426950408889634
HS = 20
HPW = 7
NW = 5
BQ = 512
BK = 128
G = 8
FC = 512
FU = 3
f32, bf16, i32 = jnp.float32, jnp.bfloat16, jnp.int32

NK = S // BK
NGRP = H // G
GR = HS * G
NQB = S // BQ
HP = HS * H
NC = F // FC
QSCALE = float(LOG2E / np.sqrt(DH))


def _ln_t(xT):
    m = jnp.sum(xT, axis=0, keepdims=True) * (1.0 / D)
    xc = xT - m
    v = jnp.sum(xc * xc, axis=0, keepdims=True) * (1.0 / D)
    return xc * jax.lax.rsqrt(v + EPS)


def _mish(h):
    t = jnp.exp2(jnp.minimum(h, 20.0) * LOG2E)
    n = t * (t + 2.0)
    return h * (n / (n + 2.0))


def _nn(a, b):
    return jnp.dot(a, b, preferred_element_type=f32)


def _nt(a, b):
    return jax.lax.dot_general(a, b, (((1,), (1,)), ((), ())), preferred_element_type=f32)


def _make():
    V = pltpu.VMEM
    scratch = dict(
        xT_s=V((D, S), bf16),
        wqkv_s=V((D, 3 * D), bf16),
        wo_s=V((D, D), bf16),
        w1_s=V((D, F), bf16),
        w2T_s=V((D, F), bf16),
        wqk_s=V((D, 2 * NW * 128), bf16),
        wvT_s=V((D, D), bf16),
        woT_s=V((D, HP), bf16),
        tmp_s=V((HP, D), f32),
        b1_s=V((8, F), f32),
        q_s=V((H, S // 2, 128), i32),
        k_s=V((NW, S // 2, 128), i32),
        vt_s=V((NGRP, GR, S), f32),
        ot_s=V((NGRP, GR, BQ), f32),
        acc_s=V((D, BQ), f32),
        sc_s=V((BK, BQ), f32),
        mc_s=V((8, BQ), f32),
        xn_s=V((NQB, BQ, D), bf16),
        xnT_s=V((NQB, D, BQ), bf16),
        b1r_s=V((F // 128, 128), bf16),
    )
    names = list(scratch)

    def kernel(xT_hbm, wqkv_hbm, wo_hbm, w1_hbm, b1_hbm, w2T_hbm, out_ref, *rest):
        sems = rest[-1]
        r = dict(zip(names, rest[:-1]))
        xT_s, wqkv_s, wo_s, w1_s, w2T_s, wqk_s, wvT_s, woT_s, tmp_s, b1_s = (
            r[n] for n in ("xT_s", "wqkv_s", "wo_s", "w1_s", "w2T_s", "wqk_s", "wvT_s", "woT_s", "tmp_s", "b1_s"))
        q_s, k_s, vt_s, ot_s, acc_s, sc_s, mc_s, xn_s, xnT_s, b1r_s = (
            r[n] for n in ("q_s", "k_s", "vt_s", "ot_s", "acc_s", "sc_s", "mc_s", "xn_s", "xnT_s", "b1r_s"))
        i = pl.program_id(0)

        def cp_x(b):
            return pltpu.make_async_copy(xT_hbm.at[:, pl.ds(b * BQ, BQ)], xT_s.at[:, pl.ds(b * BQ, BQ)], sems.at[b])
        cp_wqk = pltpu.make_async_copy(wqkv_hbm.at[:, pl.ds(0, 2 * D)], wqkv_s.at[:, pl.ds(0, 2 * D)], sems.at[NQB])
        cp_wv = pltpu.make_async_copy(wqkv_hbm.at[:, pl.ds(2 * D, D)], wqkv_s.at[:, pl.ds(2 * D, D)], sems.at[NQB + 1])
        cp_wo = pltpu.make_async_copy(wo_hbm, wo_s, sems.at[NQB + 2])
        cp_w1 = pltpu.make_async_copy(w1_hbm, w1_s, sems.at[NQB + 3])
        cp_w2 = pltpu.make_async_copy(w2T_hbm, w2T_s, sems.at[NQB + 4])
        cp_b1 = pltpu.make_async_copy(b1_hbm, b1r_s, sems.at[NQB + 5])

        @pl.when(i == 0)
        def _prologue():
            def ln1(b):
                r0 = pl.multiple_of(b * BQ, BQ)
                xnT = _ln_t(xT_s[:, pl.ds(r0, BQ)].astype(f32))
                xn_s[b] = xnT.T.astype(bf16)
                xnT_s[b] = xnT.astype(bf16)

            def windows():
                tiles = {}

                def tile(a):
                    if a not in tiles:
                        tiles[a] = pltpu.bitcast(wqkv_s[:, a * 128:(a + 1) * 128], i32)
                    return tiles[a]
                lane = jax.lax.broadcasted_iota(i32, (D // 2, 128), 1)
                for t in range(2):
                    for g in range(NW):
                        a, off = divmod(D * t + HPW * DH * g, 128)
                        if off == 0:
                            w = tile(a)
                        else:
                            w = pltpu.roll(jnp.where(lane >= off, tile(a), tile(a + 1)), 128 - off, 1)
                        wqk_s[:, (NW * t + g) * 128:(NW * t + g + 1) * 128] = pltpu.bitcast(w, bf16)

            def vproj(b):
                r0 = pl.multiple_of(b * BQ, BQ)
                vT = _nn(wvT_s[...], xnT_s[b])
                for h in range(H):
                    j, hh = divmod(h, G)
                    vt_s[j, HS * hh:HS * hh + DH, pl.ds(r0, BQ)] = vT[DH * h:DH * h + DH, :]

            def qkproj(b):
                qk = _nn(xn_s[b], wqk_s[...])
                r2 = pl.multiple_of(b * (BQ // 2), BQ // 2)
                lane = jax.lax.broadcasted_iota(i32, (BQ // 2, 128), 1)
                for g in range(NW):
                    qg = pltpu.bitcast((qk[:, g * 128:(g + 1) * 128] * QSCALE).astype(bf16), i32)
                    for h in range(g * HPW, min(H, (g + 1) * HPW)):
                        c = (h - g * HPW) * DH
                        q_s[h, pl.ds(r2, BQ // 2), :] = jnp.where((lane >= c) & (lane < c + DH), qg, 0)
                    kg = qk[:, (NW + g) * 128:(NW + g + 1) * 128].astype(bf16)
                    k_s[g, pl.ds(r2, BQ // 2), :] = pltpu.bitcast(kg, i32)

            def wo_prep():
                wof = wo_s[...].astype(f32)
                for h in range(H):
                    tmp_s[HS * h:HS * h + DH, :] = wof[DH * h:DH * h + DH, :]
                woT_s[...] = tmp_s[...].T.astype(bf16)
                for c in range(F // 128):
                    b1_s[:, c * 128:(c + 1) * 128] = jnp.broadcast_to(b1r_s[c:c + 1, :].astype(f32), (8, 128))

            cp_x(0).start()
            cp_wv.start()
            for b in range(1, NQB):
                cp_x(b).start()
            cp_wqk.start()
            cp_wo.start()
            cp_b1.start()
            cp_w1.start()
            cp_w2.start()
            two = jnp.where(jax.lax.broadcasted_iota(i32, (2, S), 0) == 0, 1.0, 0.0)
            for h in range(H):
                j, hh = divmod(h, G)
                vt_s[j, HS * hh + DH:HS * hh + HS, :] = two
                tmp_s[HS * h + DH:HS * h + HS, :] = jnp.zeros((HS - DH, D), f32)
            cp_x(0).wait()
            ln1(0)
            cp_wv.wait()
            wvT_s[...] = wqkv_s[:, 2 * D:3 * D].astype(f32).T.astype(bf16)

            def vloop(b, c):
                cp_x(b + 1).wait()
                vproj(b)
                ln1(b + 1)
                return c

            def qkloop(b, c):
                qkproj(b)
                return c

            jax.lax.fori_loop(0, NQB - 1, vloop, 0)
            cp_wqk.wait()
            vproj(NQB - 1)
            windows()
            jax.lax.fori_loop(0, NQB - 1, qkloop, 0)
            cp_wo.wait()
            cp_b1.wait()
            qkproj(NQB - 1)
            wo_prep()

        q0 = pl.multiple_of(i * BQ, BQ)
        q2 = pl.multiple_of(i * (BQ // 2), BQ // 2)

        def head(j, hh):
            h = j * G + hh
            return h, (h * 37) >> 8

        def scores(hg, r2, kb):
            h, g = hg
            q = pltpu.bitcast(q_s[h, pl.ds(r2, BQ // 2), :], bf16)
            k = pltpu.bitcast(k_s[g, kb * (BK // 2):(kb + 1) * (BK // 2), :], bf16)
            sT = _nt(k, q)
            return sT, jnp.max(sT, axis=0, keepdims=True)

        def probs(kb, smx, m_run):
            sT, mx = smx
            if kb == 0:
                m_new, alpha = mx, None
            else:
                m_new = jnp.maximum(m_run, mx)
                alpha = jnp.exp2(m_run - m_new)
            return jnp.exp2(sT - m_new), alpha, m_new

        def pv(j, hh, kb, p, alpha, acc):
            st = 8 * ((HS * hh) // 8)
            off = HS * hh - st
            r = _nn(vt_s[j, st:st + 24, kb * BK:(kb + 1) * BK], p)
            acc = r if kb == 0 else acc * alpha + r
            if kb == NK - 1:
                l = acc[off + DH:off + DH + 1, :]
                ot_s[j, HS * hh:HS * hh + HS, :] = acc[off:off + HS, :] * pltpu.reciprocal(l, approx=False)
            return acc

        N = G * NK

        def group(j, c):
            last = j == NGRP - 1
            jn = jnp.where(last, 0, j + 1)
            q2n = pl.multiple_of(jnp.minimum(i + last.astype(i32), NQB - 1) * (BQ // 2), BQ // 2)
            heads = {}

            def step(n):
                key = n // NK
                if key not in heads:
                    heads[key] = (head(j, key), q2) if key < G else (head(jn, 0), q2n)
                return scores(*heads[key], n % NK)
            first = (sc_s[...], mc_s[0:1, :])
            As = {1: step(1)}
            p, alpha, m_run = probs(0, first, None)
            Bs = {0: (p, alpha)}
            acc = None
            for n in range(N):
                if n + 2 <= N:
                    As[n + 2] = step(n + 2)
                if n + 1 < N:
                    p, alpha, m_run = probs((n + 1) % NK, As.pop(n + 1), m_run)
                    Bs[n + 1] = (p, alpha)
                acc = pv(j, n // NK, n % NK, *Bs.pop(n), acc)
            sT, mx = As.pop(N)
            sc_s[...] = sT
            mc_s[0:1, :] = mx
            return c

        @pl.when(i == 0)
        def _():
            sT, mx = scores(head(0, 0), 0, 0)
            sc_s[...] = sT
            mc_s[0:1, :] = mx
        jax.lax.fori_loop(0, NGRP, group, 0)

        @pl.when(i == 0)
        def _():
            cp_w1.wait()
            cp_w2.wait()

        oT = ot_s[...].reshape(HP, BQ).astype(bf16)
        hT = xT_s[:, pl.ds(q0, BQ)].astype(f32) + _nn(woT_s[...], oT)
        y = _ln_t(hT).T.astype(bf16)
        acc_s[...] = hT

        def ffn1(c0):
            h1 = _nn(y, w1_s[:, pl.ds(c0, FC)])
            h1 = (h1.reshape(BQ // 8, 8, FC) + b1_s[:, pl.ds(c0, FC)][None]).reshape(BQ, FC)
            return _mish(h1).astype(bf16)

        def ffn(it, c):
            base = it * (FU * FC)
            a = ffn1(pl.multiple_of(base, FC))
            acc = acc_s[...]
            for u in range(FU):
                a_next = ffn1(pl.multiple_of(base + (u + 1) * FC, FC)) if u + 1 < FU else None
                acc = acc + _nt(w2T_s[:, pl.ds(pl.multiple_of(base + u * FC, FC), FC)], a)
                a = a_next
            acc_s[...] = acc
            out_ref[...] = acc.astype(bf16)
            return c
        jax.lax.fori_loop(0, NC // FU, ffn, 0)

    hbm = pl.BlockSpec(memory_space=pltpu.HBM)
    call = pl.pallas_call(
        kernel,
        grid=(NQB,),
        in_specs=[hbm] * 6,
        out_specs=pl.BlockSpec((D, BQ), lambda i: (0, i)),
        out_shape=jax.ShapeDtypeStruct((D, S), bf16),
        scratch_shapes=[scratch[n] for n in names] + [pltpu.SemaphoreType.DMA((NQB + 6,))],
        compiler_params=pltpu.CompilerParams(
            dimension_semantics=("arbitrary",),
            vmem_limit_bytes=100 * 1024 * 1024,
        ),
    )

    def fn(A_x, A_wqkv, A_wo, B_x, B_w1, B_b1, B_w2):
        outT = call(A_x.reshape(S, D).T, A_wqkv, A_wo, B_w1, B_b1.reshape(F // 128, 128), B_w2.T)
        return outT.T.reshape(1, S, D)
    return fn


_impl = _make()


@jax.jit
def pallas_sequential_preLN__mha_block__dense_activation_mish__prompt_kernel(
    A_x: jax.Array,
    A_wqkv: jax.Array,
    A_wo: jax.Array,
    B_x: jax.Array,
    B_w1: jax.Array,
    B_b1: jax.Array,
    B_w2: jax.Array,
):
    return _impl(A_x, A_wqkv, A_wo, B_x, B_w1, B_b1, B_w2)
```

```python
import numpy as np
import jax
import jax.numpy as jnp
import jax.experimental.pallas as pl
import jax.experimental.pallas.tpu as pltpu

S, D, H, DH, F = 2048, 576, 32, 18, 4608
EPS = 1e-5
LOG2E = 1.4426950408889634
HS = 20
HPW = 7
NW = 5
BQ = 512
BK = 128
G = 8
FC = 512
FU = 3
f32, bf16, i32 = jnp.float32, jnp.bfloat16, jnp.int32

NK = S // BK
NGRP = H // G
GR = HS * G
NQB = S // BQ
HP = HS * H
NC = F // FC
QSCALE = float(LOG2E / np.sqrt(DH))


def _ln_t(xT):
    m = jnp.sum(xT, axis=0, keepdims=True) * (1.0 / D)
    xc = xT - m
    v = jnp.sum(xc * xc, axis=0, keepdims=True) * (1.0 / D)
    return xc * jax.lax.rsqrt(v + EPS)


def _mish(h):
    t = jnp.exp2(jnp.minimum(h, 20.0) * LOG2E)
    n = t * (t + 2.0)
    return h * (n / (n + 2.0))


def _nn(a, b):
    return jnp.dot(a, b, preferred_element_type=f32)


def _nt(a, b):
    return jax.lax.dot_general(a, b, (((1,), (1,)), ((), ())), preferred_element_type=f32)


def _make():
    V = pltpu.VMEM
    scratch_shapes = [
        V((D, S), bf16),
        V((D, 3 * D), bf16),
        V((D, D), bf16),
        V((D, F), bf16),
        V((D, F), bf16),
        V((D, 2 * NW * 128), bf16),
        V((D, D), bf16),
        V((D, HP), bf16),
        V((HP, D), f32),
        V((8, F), f32),
        V((H, S // 2, 128), i32),
        V((NW, S // 2, 128), i32),
        V((NGRP, GR, S), f32),
        V((NGRP, GR, BQ), f32),
        V((D, BQ), f32),
        V((BK, BQ), f32),
        V((8, BQ), f32),
        V((NQB, BQ, D), bf16),
        V((NQB, D, BQ), bf16),
        V((F // 128, 128), bf16),
        pltpu.SemaphoreType.DMA((NQB + 6,)),
    ]

    def kernel(xT_hbm, wqkv_hbm, wo_hbm, w1_hbm, b1_hbm, w2T_hbm, out_ref,
               xT_s, wqkv_s, wo_s, w1_s, w2T_s, wqk_s, wvT_s, woT_s, tmp_s, b1_s,
               q_s, k_s, vt_s, ot_s, acc_s, sc_s, mc_s, xn_s, xnT_s, b1r_s, sems):
        i = pl.program_id(0)

        def cp_x(b):
            return pltpu.make_async_copy(xT_hbm.at[:, pl.ds(b * BQ, BQ)], xT_s.at[:, pl.ds(b * BQ, BQ)], sems.at[b])
        cp_wqk = pltpu.make_async_copy(wqkv_hbm.at[:, pl.ds(0, 2 * D)], wqkv_s.at[:, pl.ds(0, 2 * D)], sems.at[NQB])
        cp_wv = pltpu.make_async_copy(wqkv_hbm.at[:, pl.ds(2 * D, D)], wqkv_s.at[:, pl.ds(2 * D, D)], sems.at[NQB + 1])
        cp_wo = pltpu.make_async_copy(wo_hbm, wo_s, sems.at[NQB + 2])
        cp_w1 = pltpu.make_async_copy(w1_hbm, w1_s, sems.at[NQB + 3])
        cp_w2 = pltpu.make_async_copy(w2T_hbm, w2T_s, sems.at[NQB + 4])
        cp_b1 = pltpu.make_async_copy(b1_hbm, b1r_s, sems.at[NQB + 5])

        @pl.when(i == 0)
        def _prologue():
            def ln1(b):
                r0 = pl.multiple_of(b * BQ, BQ)
                xnT = _ln_t(xT_s[:, pl.ds(r0, BQ)].astype(f32))
                xn_s[b] = xnT.T.astype(bf16)
                xnT_s[b] = xnT.astype(bf16)

            def windows():
                tiles = {}

                def tile(a):
                    if a not in tiles:
                        tiles[a] = pltpu.bitcast(wqkv_s[:, a * 128:(a + 1) * 128], i32)
                    return tiles[a]
                lane = jax.lax.broadcasted_iota(i32, (D // 2, 128), 1)
                for t in range(2):
                    for g in range(NW):
                        a, off = divmod(D * t + HPW * DH * g, 128)
                        if off == 0:
                            w = tile(a)
                        else:
                            w = pltpu.roll(jnp.where(lane >= off, tile(a), tile(a + 1)), 128 - off, 1)
                        wqk_s[:, (NW * t + g) * 128:(NW * t + g + 1) * 128] = pltpu.bitcast(w, bf16)

            def vproj(b):
                r0 = pl.multiple_of(b * BQ, BQ)
                vT = _nn(wvT_s[...], xnT_s[b])
                for h in range(H):
                    j, hh = divmod(h, G)
                    vt_s[j, HS * hh:HS * hh + DH, pl.ds(r0, BQ)] = vT[DH * h:DH * h + DH, :]

            def qkproj(b):
                qk = _nn(xn_s[b], wqk_s[...])
                r2 = pl.multiple_of(b * (BQ // 2), BQ // 2)
                lane = jax.lax.broadcasted_iota(i32, (BQ // 2, 128), 1)
                for g in range(NW):
                    qg = pltpu.bitcast((qk[:, g * 128:(g + 1) * 128] * QSCALE).astype(bf16), i32)
                    for h in range(g * HPW, min(H, (g + 1) * HPW)):
                        c = (h - g * HPW) * DH
                        q_s[h, pl.ds(r2, BQ // 2), :] = jnp.where((lane >= c) & (lane < c + DH), qg, 0)
                    kg = qk[:, (NW + g) * 128:(NW + g + 1) * 128].astype(bf16)
                    k_s[g, pl.ds(r2, BQ // 2), :] = pltpu.bitcast(kg, i32)

            def wo_prep():
                wof = wo_s[...].astype(f32)
                for h in range(H):
                    tmp_s[HS * h:HS * h + DH, :] = wof[DH * h:DH * h + DH, :]
                woT_s[...] = tmp_s[...].T.astype(bf16)
                for c in range(F // 128):
                    b1_s[:, c * 128:(c + 1) * 128] = jnp.broadcast_to(b1r_s[c:c + 1, :].astype(f32), (8, 128))

            cp_x(0).start()
            cp_wv.start()
            for b in range(1, NQB):
                cp_x(b).start()
            cp_wqk.start()
            cp_wo.start()
            cp_b1.start()
            cp_w1.start()
            cp_w2.start()
            two = jnp.where(jax.lax.broadcasted_iota(i32, (2, S), 0) == 0, 1.0, 0.0)
            for h in range(H):
                j, hh = divmod(h, G)
                vt_s[j, HS * hh + DH:HS * hh + HS, :] = two
                tmp_s[HS * h + DH:HS * h + HS, :] = jnp.zeros((HS - DH, D), f32)
            cp_x(0).wait()
            ln1(0)
            cp_wv.wait()
            wvT_s[...] = wqkv_s[:, 2 * D:3 * D].astype(f32).T.astype(bf16)

            def vloop(b, c):
                cp_x(b + 1).wait()
                vproj(b)
                ln1(b + 1)
                return c

            def qkloop(b, c):
                qkproj(b)
                return c

            jax.lax.fori_loop(0, NQB - 1, vloop, 0)
            cp_wqk.wait()
            vproj(NQB - 1)
            windows()
            jax.lax.fori_loop(0, NQB - 1, qkloop, 0)
            cp_wo.wait()
            cp_b1.wait()
            qkproj(NQB - 1)
            wo_prep()

        q0 = pl.multiple_of(i * BQ, BQ)
        q2 = pl.multiple_of(i * (BQ // 2), BQ // 2)

        def head(j, hh):
            h = j * G + hh
            return h, (h * 37) >> 8

        def scores(hg, r2, kb):
            h, g = hg
            q = pltpu.bitcast(q_s[h, pl.ds(r2, BQ // 2), :], bf16)
            k = pltpu.bitcast(k_s[g, kb * (BK // 2):(kb + 1) * (BK // 2), :], bf16)
            sT = _nt(k, q)
            return sT, jnp.max(sT, axis=0, keepdims=True)

        def probs(kb, smx, m_run):
            sT, mx = smx
            if kb == 0:
                m_new, alpha = mx, None
            else:
                m_new = jnp.maximum(m_run, mx)
                alpha = jnp.exp2(m_run - m_new)
            return jnp.exp2(sT - m_new), alpha, m_new

        def pv(j, hh, kb, p, alpha, acc):
            st = 8 * ((HS * hh) // 8)
            off = HS * hh - st
            r = _nn(vt_s[j, st:st + 24, kb * BK:(kb + 1) * BK], p)
            acc = r if kb == 0 else acc * alpha + r
            if kb == NK - 1:
                l = acc[off + DH:off + DH + 1, :]
                ot_s[j, HS * hh:HS * hh + HS, :] = acc[off:off + HS, :] * pltpu.reciprocal(l, approx=False)
            return acc

        N = G * NK

        def group(j, c):
            last = j == NGRP - 1
            jn = jnp.where(last, 0, j + 1)
            q2n = pl.multiple_of(jnp.minimum(i + last.astype(i32), NQB - 1) * (BQ // 2), BQ // 2)
            heads = {}

            def step(n):
                key = n // NK
                if key not in heads:
                    heads[key] = (head(j, key), q2) if key < G else (head(jn, 0), q2n)
                return scores(*heads[key], n % NK)
            first = (sc_s[...], mc_s[0:1, :])
            As = {1: step(1)}
            p, alpha, m_run = probs(0, first, None)
            Bs = {0: (p, alpha)}
            acc = None
            for n in range(N):
                if n + 2 <= N:
                    As[n + 2] = step(n + 2)
                if n + 1 < N:
                    p, alpha, m_run = probs((n + 1) % NK, As.pop(n + 1), m_run)
                    Bs[n + 1] = (p, alpha)
                acc = pv(j, n // NK, n % NK, *Bs.pop(n), acc)
            sT, mx = As.pop(N)
            sc_s[...] = sT
            mc_s[0:1, :] = mx
            return c

        @pl.when(i == 0)
        def _():
            sT, mx = scores(head(0, 0), 0, 0)
            sc_s[...] = sT
            mc_s[0:1, :] = mx
        jax.lax.fori_loop(0, NGRP, group, 0)

        @pl.when(i == 0)
        def _():
            cp_w1.wait()
            cp_w2.wait()

        oT = ot_s[...].reshape(HP, BQ).astype(bf16)
        hT = xT_s[:, pl.ds(q0, BQ)].astype(f32) + _nn(woT_s[...], oT)
        y = _ln_t(hT).T.astype(bf16)
        acc_s[...] = hT

        def ffn1(c0):
            h1 = _nn(y, w1_s[:, pl.ds(c0, FC)])
            h1 = (h1.reshape(BQ // 8, 8, FC) + b1_s[:, pl.ds(c0, FC)][None]).reshape(BQ, FC)
            return _mish(h1).astype(bf16)

        def ffn(it, c):
            base = it * (FU * FC)
            a = ffn1(pl.multiple_of(base, FC))
            acc = acc_s[...]
            for u in range(FU):
                a_next = ffn1(pl.multiple_of(base + (u + 1) * FC, FC)) if u + 1 < FU else None
                acc = acc + _nt(w2T_s[:, pl.ds(pl.multiple_of(base + u * FC, FC), FC)], a)
                a = a_next
            acc_s[...] = acc
            out_ref[...] = acc.astype(bf16)
            return c
        jax.lax.fori_loop(0, NC // FU, ffn, 0)

    hbm = pl.BlockSpec(memory_space=pltpu.HBM)
    call = pl.pallas_call(
        kernel,
        grid=(NQB,),
        in_specs=[hbm] * 6,
        out_specs=pl.BlockSpec((D, BQ), lambda i: (0, i)),
        out_shape=jax.ShapeDtypeStruct((D, S), bf16),
        scratch_shapes=scratch_shapes,
        compiler_params=pltpu.CompilerParams(
            dimension_semantics=("arbitrary",),
            vmem_limit_bytes=100 * 1024 * 1024,
        ),
    )

    def fn(A_x, A_wqkv, A_wo, B_x, B_w1, B_b1, B_w2):
        outT = call(A_x.reshape(S, D).T, A_wqkv, A_wo, B_w1, B_b1.reshape(F // 128, 128), B_w2.T)
        return outT.T.reshape(1, S, D)
    return fn


_impl = _make()


@jax.jit
def pallas_sequential_preLN__mha_block__dense_activation_mish__prompt_kernel(
    A_x: jax.Array,
    A_wqkv: jax.Array,
    A_wo: jax.Array,
    B_x: jax.Array,
    B_w1: jax.Array,
    B_b1: jax.Array,
    B_w2: jax.Array,
):
    return _impl(A_x, A_wqkv, A_wo, B_x, B_w1, B_b1, B_w2)
```
